```python
import os as _os
_os.environ.setdefault('JAX_PLATFORMS', 'cpu')
import jax
import jax.numpy as jnp

def _softmax(x, axis=-1):
    return jax.nn.softmax(x, axis=axis)

def _gelu(x):
    return jax.nn.gelu(x, approximate=True)

def _silu(x):
    return jax.nn.silu(x)

def _sigmoid(x):
    return jax.nn.sigmoid(x)

def _layernorm(x, axis=-1, eps=1e-05):
    m = jnp.mean(x, axis=axis, keepdims=True)
    v = jnp.var(x, axis=axis, keepdims=True)
    return (x - m) / jnp.sqrt(v + eps)

def _scatter_add(tgt, idx, src, axis=0):
    return tgt.at[idx].add(src)

def _segment_sum(src, seg, n):
    return jax.ops.segment_sum(src, seg, n)

class _Rng:

    def __init__(self, key):
        self._k = key

    def _next(self):
        self._k, sub = jax.random.split(self._k)
        return sub

    def normal(self, shape):
        return jax.random.normal(self._next(), shape, dtype=jnp.bfloat16)

    def randint(self, lo, hi, shape):
        return jax.random.randint(self._next(), shape, lo, hi, dtype=jnp.int32)

    def uniform(self, shape, lo=0.0, hi=1.0):
        return jax.random.uniform(self._next(), shape, jnp.bfloat16, lo, hi)

    def permutation(self, n):
        return jax.random.permutation(self._next(), n)
kernel_name = 'adaLN_cond__sliding_local_dilated__dense_activation_relu__prompt'

def setup_inputs():
    _rng = _Rng(jax.random.key(int.from_bytes(__import__("os").urandom(4), "little")))
    _w = lambda a: (lambda t: t.astype(jnp.bfloat16) if jnp.issubdtype(t.dtype, jnp.floating) else t)(jnp.asarray(a))

    def _A_setup():
        B, S, D = (1, 2048, 576)
        return {'x': _w((lambda *s: _rng.normal(s) * 0.05)(B, S, D)), 'wqkv': _w((lambda *s: _rng.normal(s) * 0.05)(D, 3 * D)), 'wo': _w((lambda *s: _rng.normal(s) * 0.05)(D, D))}
    _A_in = _A_setup()

    def _B_setup():
        B, S, D, Dff = (1, 2048, 576, 4608)
        return {'x': _w((lambda *s: _rng.normal(s) * 0.05)(B, S, D)), 'w1': _w((lambda *s: _rng.normal(s) * 0.05)(D, Dff)), 'w2': _w((lambda *s: _rng.normal(s) * 0.05)(Dff, D))}
    _B_in = _B_setup()
    return {'A_x': _A_in['x'], 'A_wqkv': _A_in['wqkv'], 'A_wo': _A_in['wo'], 'B_x': _B_in['x'], 'B_w1': _B_in['w1'], 'B_w2': _B_in['w2'], 'c': _w((lambda *s: _rng.normal(s) * 0.05)(1, 576) * 8.0), 'w_mod': _w((lambda *s: _rng.normal(s) * 0.05)(576, 6 * 576) * 576 ** (-0.5) * 8.0)}

def reference(A_x, A_wqkv, A_wo, B_x, B_w1, B_w2, c, w_mod):

    def _A_ref(x, wqkv, wo):
        B, S, D = x.shape
        H = 32
        Dh = D // H
        W, dil = (8, 2)
        qkv = (lambda x, *d: x.transpose(*d))((x @ wqkv).reshape(B, S, 3, H, Dh), 2, 0, 3, 1, 4)
        q, k, v = (qkv[0], qkv[1], qkv[2])
        scale = Dh ** (-0.5)
        pos = jnp.arange(S)
        off = jnp.arange(W) * dil
        idx = pos[:, None] - off[None, :]
        mask = idx >= 0
        idx_c = jnp.where(mask, idx, 0).reshape(-1)
        kg = k[:, :, idx_c, :].reshape(B, H, S, W, Dh)
        vg = v[:, :, idx_c, :].reshape(B, H, S, W, Dh)
        logits = jnp.einsum('bhsd,bhswd->bhsw', q, kg) * scale
        logits = jnp.where(mask[None, None, :, :], logits, -1000000000.0)
        attn = _softmax(logits, axis=-1)
        o = jnp.einsum('bhsw,bhswd->bhsd', attn, vg)
        return (lambda x, *d: x.transpose(*d))(o, 0, 2, 1, 3).reshape(B, S, D) @ wo

    def _B_ref(x, w1, w2):
        h = jnp.einsum('bsd,df->bsf', x, w1)
        zero = jnp.zeros_like(h)
        h = jnp.maximum(h, zero)
        return jnp.einsum('bsf,fd->bsd', h, w2)
    x = A_x
    mod = (_silu(c) @ w_mod).reshape(c.shape[0], 6, 1, -1)
    sa, ca, ga, sb, cb, gb = (mod[:, 0].copy(), mod[:, 1].copy(), mod[:, 2].copy(), mod[:, 3].copy(), mod[:, 4].copy(), mod[:, 5].copy())
    h = _layernorm(x, axis=-1) * (1 + ca) + sa
    x = x + ga * _A_ref(h, A_wqkv, A_wo)
    h = _layernorm(x, axis=-1) * (1 + cb) + sb
    x = x + gb * _B_ref(h, B_w1, B_w2)
    return x
```

```python
import functools
import jax
import jax.numpy as jnp
import numpy as np
from jax import lax
import jax.experimental.pallas as pl
import jax.experimental.pallas.tpu as pltpu

S, D, H, DH, W, DIL, DFF = 2048, 576, 32, 18, 8, 2, 4608
TB = 256
NB = S // TB
TF = 256
NF = S // TF
HF = DFF // 2
NJ = DH // 2
SCALE = float(DH ** -0.5)
EPS = 1e-5
NEG = -1e9
f32, bf16, u32, i32 = jnp.float32, jnp.bfloat16, jnp.uint32, jnp.int32
RSTEP = 8
PROFILE = False


def _scope(name):
    import contextlib
    return jax.named_scope(name) if PROFILE else contextlib.nullcontext()


def _ds(start, size, mult=128):
    if isinstance(start, int):
        return pl.ds(start, size)
    return pl.ds(pl.multiple_of(start, mult), size)


def _unp(x, i):
    return pltpu.unpack_elementwise(x, index=i, packed_dtype=bf16, unpacked_dtype=f32)


def _pk(a, b):
    return pltpu.pack_elementwise([a, b], packed_dtype=bf16)


def _ln(xf, a, b):
    m = jnp.sum(xf, axis=0, keepdims=True) * (1.0 / D)
    xc = xf - m
    v = jnp.sum(xc * xc, axis=0, keepdims=True) * (1.0 / D)
    return xc * lax.rsqrt(v + EPS) * a + b


def _kernel(xT_hbm, wqkv_hbm, wo_hbm, w1_hbm, w2T_hbm, c_hbm, wm_hbm, outT_hbm,
            x_s, wqkv_s, wo_s, w1_s, w2T_s, c_s, wm_s, tmp_s, wqT_s, woT_s, modc_s,
            hT0, hT1, qb0, qb1, o_s, x1_s, xo_s, xr_s, hb_s, w1c_s, w2c_s, out_s, sems, osems):
    hT = (hT0, hT1)
    qb = (qb0, qb1)

    def cp(i, src, dst):
        return pltpu.make_async_copy(src, dst, sems.at[i])
    NM1 = 2 * D
    X0 = 2 * TB
    d_c = cp(0, c_hbm, c_s)
    d_wm1 = cp(1, wm_hbm.at[:, 0:NM1], wm_s.at[:, 0:NM1])
    d_x0 = cp(2, xT_hbm.at[:, 0:X0], x_s.at[:, 0:X0])
    d_wqkv = cp(3, wqkv_hbm, wqkv_s)
    d_x1 = cp(4, xT_hbm.at[:, X0:S], x_s.at[:, X0:S])
    d_wm2 = cp(5, wm_hbm.at[:, NM1:6 * D], wm_s.at[:, NM1:6 * D])
    d_wo = cp(6, wo_hbm, wo_s)
    d_w1 = cp(7, w1_hbm.bitcast(u32), w1_s)
    d_w2 = cp(8, w2T_hbm.bitcast(u32), w2T_s)
    for d in (d_c, d_wm1, d_x0, d_wqkv, d_x1, d_wm2, d_wo, d_w1, d_w2):
        d.start()

    lane = lax.broadcasted_iota(i32, (8, 128), 1)

    def compute_mod(lo, hi):
        cf = c_s[...].astype(f32)
        sc = (cf * jax.nn.sigmoid(cf)).astype(bf16)
        sc16 = jnp.broadcast_to(sc, (16, D))
        mod = jnp.dot(sc16, wm_s[:, lo:hi], preferred_element_type=f32)
        row = mod[0:1, :]
        for n in range((hi - lo) // 128):
            blk = jnp.broadcast_to(row[:, n * 128:(n + 1) * 128], (128, 128))
            modc_s[lo + n * 128: lo + (n + 1) * 128, :] = blk.T

    def modv(k):
        return modc_s[k * D:(k + 1) * D, :]

    def ln1(base, slot):
        for cc in range(TB // 128):
            xf = x_s[:, _ds(base + cc * 128, 128)].astype(f32)
            hT[slot][:, cc * 128:(cc + 1) * 128] = _ln(xf, modv(1), modv(0)).astype(bf16)

    def qproj(slot):
        wt = pltpu.bitcast(wqT_s[...], bf16)
        r = jnp.dot(wt, hT[slot][...], preferred_element_type=f32).astype(bf16)
        qb[slot][:, 128:128 + TB] = pltpu.bitcast(r, u32)
        qb[1 - slot][288:864, 0:128] = qb[slot][288:864, TB:TB + 128]

    def attn_chunk(base, slot, cc):
        qr = qb[slot]
        cur = pl.ds(128 + cc * 128, 128)
        prev = pl.ds(cc * 128, 128)
        pos = lane + (base + cc * 128)
        for hg in range(4):
            acc = [None] * W
            for j in range(NJ):
                r = j * 32 + hg * 8
                qw = qr[r:r + 8, cur]
                q0, q1 = _unp(qw, 0), _unp(qw, 1)
                kc = qr[288 + r:288 + r + 8, cur]
                kp = qr[288 + r:288 + r + 8, prev]
                for w in range(W):
                    ks = kc if w == 0 else pltpu.roll(jnp.where(lane < 128 - DIL * w, kc, kp), DIL * w, axis=1)
                    p = q0 * _unp(ks, 0) + q1 * _unp(ks, 1)
                    acc[w] = p if acc[w] is None else acc[w] + p
            lg = [acc[0] * SCALE] + [jnp.where(pos >= DIL * w, acc[w] * SCALE, NEG) for w in range(1, W)]
            m = lg[0]
            for w in range(1, W):
                m = jnp.maximum(m, lg[w])
            e = [jnp.exp(l - m) for l in lg]
            s = e[0]
            for w in range(1, W):
                s = s + e[w]
            rinv = 1.0 / s
            p = [x * rinv for x in e]
            for j in range(NJ):
                r = j * 32 + hg * 8
                vc = qr[576 + r:576 + r + 8, cur]
                vp = qr[576 + r:576 + r + 8, prev]
                o0 = o1 = None
                for w in range(W):
                    vs = vc if w == 0 else pltpu.roll(jnp.where(lane < 128 - DIL * w, vc, vp), DIL * w, axis=1)
                    t0 = p[w] * _unp(vs, 0)
                    t1 = p[w] * _unp(vs, 1)
                    o0 = t0 if o0 is None else o0 + t0
                    o1 = t1 if o1 is None else o1 + t1
                o_s[r:r + 8, _ds(base + cc * 128, 128)] = _pk(o0, o1)

    def attn(base, slot):
        for cc in range(TB // 128):
            attn_chunk(base, slot, cc)

    def oproj(base):
        wt = pltpu.bitcast(woT_s[...], bf16)
        ov = pltpu.bitcast(o_s[:, _ds(base, TB)], bf16)
        att = jnp.dot(wt, ov, preferred_element_type=f32)
        ga = modv(2)
        for cc in range(TB // 128):
            c1 = _ds(base + cc * 128, 128)
            x1_s[:, c1] = x_s[:, c1].astype(f32) + ga * att[:, cc * 128:(cc + 1) * 128]

    def bc(v):
        return pltpu.bitcast(v, bf16)

    def ln2(blk):
        base = blk * TF
        hh = [_ln(x1_s[:, _ds(base + cc * 128, 128)], modv(4), modv(3)) for cc in range(2)]
        x11, x12, x21, x22 = hh[0][0:256], hh[0][256:512], hh[1][0:256], hh[1][256:512]
        ops = (x11 + x22, x21 + x22, x11, x22, x11 + x12, x21 - x11, x12 - x22)
        for k in range(7):
            xo_s[_ds(blk * 448 + k * 64, 64, 64), :] = pltpu.bitcast(ops[k].astype(bf16).T, u32)
        for cc in range(2):
            xr_s[_ds(blk * 128 + cc * 64, 64, 64), 0:64] = pltpu.bitcast(hh[cc][512:D].astype(bf16).T, u32)

    def ffn(blk, slot):
        base = blk * TF
        TN = 128
        xs = [bc(xo_s[_ds(blk * 448 + k * 64, 64, 64), :]) for k in range(7)]
        xr = bc(xr_s[_ds(blk * 128, 128, 128), :])[:, 0:64]
        for j in range(HF // TN):
            c1 = slice(j * TN, (j + 1) * TN)
            c2 = slice(HF + j * TN, HF + (j + 1) * TN)
            wk = (w1c_s[0:128, c1], w1_s[0:128, c1], w1c_s[128:256, c1], w1c_s[256:384, c1],
                  w1_s[128:256, c2], w1c_s[384:512, c1], w1c_s[512:640, c1])
            m = [jnp.dot(xs[k], bc(wk[k]), preferred_element_type=f32) for k in range(7)]
            r1 = jnp.dot(xr, bc(w1_s[256:288, c1]), preferred_element_type=f32)
            r2 = jnp.dot(xr, bc(w1_s[256:288, c2]), preferred_element_type=f32)
            h11 = m[0] + m[3] - m[4] + m[6] + r1[0:128]
            h12 = m[2] + m[4] + r2[0:128]
            h21 = m[1] + m[3] + r1[128:256]
            h22 = m[0] - m[1] + m[2] + m[5] + r2[128:256]
            b11 = jnp.maximum(h11, 0.0)
            b12 = jnp.maximum(h21, 0.0)
            b21 = jnp.maximum(h12, 0.0)
            b22 = jnp.maximum(h22, 0.0)
            bs = (b11 + b22, b11, b12 - b22, b21 - b11, b22, b11 + b12, b21 + b22)
            for k in range(7):
                hb_s[k * 64:(k + 1) * 64, c1] = pltpu.bitcast(bs[k].astype(bf16), u32)
        ak = (w2c_s[0:144, :], w2c_s[144:288, :], w2T_s[0:144, 0:HF], w2T_s[144:288, HF:DFF],
              w2c_s[288:432, :], w2c_s[432:576, :], w2c_s[576:720, :])
        m = [lax.dot_general(bc(ak[k]), bc(hb_s[k * 64:(k + 1) * 64, :]), (((1,), (1,)), ((), ())),
                             preferred_element_type=f32) for k in range(7)]
        cq = ((m[0] + m[3] - m[4] + m[6], m[2] + m[4]), (m[1] + m[3], m[0] - m[1] + m[2] + m[5]))
        for r in range(2):
            rr = slice(r * 288, (r + 1) * 288)
            gb = modc_s[5 * D + r * 288:5 * D + (r + 1) * 288, :]
            for cc in range(2):
                c1 = _ds(base + cc * 128, 128)
                out_s[slot, rr, cc * 128:(cc + 1) * 128] = (x1_s[rr, c1] + gb * cq[r][cc]).astype(bf16)

    def combos(dst, src, rows, signs2, part, nparts):
        ncol = HF // 128
        for cidx in range(ncol * part // nparts, ncol * (part + 1) // nparts):
            c1 = slice(cidx * 128, (cidx + 1) * 128)
            c2 = slice(HF + cidx * 128, HF + (cidx + 1) * 128)
            for r0 in range(0, rows, RSTEP):
                ra = slice(r0, r0 + RSTEP)
                rb = slice(rows + r0, rows + r0 + RSTEP)
                quad = (src[ra, c1], src[ra, c2], src[rb, c1], src[rb, c2])
                lo = [_unp(q, 0) for q in quad]
                hi = [_unp(q, 1) for q in quad]
                for n, (ia, ib, sgn) in enumerate(signs2):
                    rd = slice(n * rows + r0, n * rows + r0 + RSTEP)
                    if sgn > 0:
                        dst[rd, c1] = _pk(lo[ia] + lo[ib], hi[ia] + hi[ib])
                    else:
                        dst[rd, c1] = _pk(lo[ia] - lo[ib], hi[ia] - hi[ib])

    def prep_w1(part=0, nparts=1):
        combos(w1c_s, w1_s, 128, ((0, 3, 1), (1, 3, -1), (2, 0, -1), (0, 1, 1), (2, 3, 1)), part, nparts)

    def prep_w2(part=0, nparts=1):
        combos(w2c_s, w2T_s, 144, ((0, 3, 1), (2, 3, 1), (0, 1, 1), (2, 0, -1), (1, 3, -1)), part, nparts)

    def prep_wqkv():
        for cidx in range(14):
            ncol = 128 if cidx < 13 else 64
            t = wqkv_s[:, cidx * 128: cidx * 128 + ncol].T
            tw = pltpu.bitcast(t, u32)
            for kt in range(5):
                kw = 128 if kt < 4 else 64
                tmp_s[kt, cidx * 64: cidx * 64 + ncol // 2, 0:kw] = tw[:, kt * 128: kt * 128 + kw]
        for which in range(3):
            for j in range(NJ):
                for kt in range(5):
                    kw = 128 if kt < 4 else 64
                    v = tmp_s[kt, pl.ds(which * 288 + j, 32, stride=NJ), :]
                    wqT_s[which * 288 + j * 32: which * 288 + (j + 1) * 32, kt * 128: kt * 128 + kw] = v[:, 0:kw]

    def prep_wo():
        wv = pltpu.bitcast(wo_s[...], u32)
        for nt in range(5):
            nw = 128 if nt < 4 else 64
            tmp_s[nt, 0:288, 0:nw] = wv[:, nt * 128: nt * 128 + nw]
        for nt in range(5):
            nw = 128 if nt < 4 else 64
            parts = [tmp_s[nt, pl.ds(j, 32, stride=NJ), :] for j in range(NJ)]
            pw = jnp.concatenate(parts, axis=0)
            pb = pltpu.bitcast(pw, bf16)
            tt = pb[:, 0:nw].T
            woT_s[nt * 64: nt * 64 + nw // 2, :] = pltpu.bitcast(tt, u32)

    qb0[288:864, 0:128] = jnp.zeros((576, 128), u32)
    with _scope("s_wait_mod"):
        d_c.wait()
        d_wm1.wait()
    compute_mod(0, NM1)
    modc_s[D:2 * D, :] = modc_s[D:2 * D, :] + 1.0
    d_x0.wait()
    ln1(0, 0)
    with _scope("s_wait_wqkv"):
        d_wqkv.wait()
    prep_wqkv()

    with _scope("s_q0"):
        qproj(0)
        ln1(TB, 1)
        d_x1.wait()
        attn(0, 0)
        qproj(1)
        ln1(2 * TB, 0)

    def body(i, par):
        attn((i - 1) * TB, 1 - par)
        qproj(par)
        nxt = jnp.minimum(i + 1, NB - 1) if not isinstance(i, int) else min(i + 1, NB - 1)
        ln1(nxt * TB, 1 - par)

    with _scope("s_p1loop"):
        @pl.loop(0, (NB - 2) // 2)
        def _(ii):
            i = 2 + 2 * ii
            body(i, 0)
            body(i + 1, 1)

    with _scope("s_p1end"):
        d_wm2.wait()
        d_wo.wait()
        compute_mod(NM1, 6 * D)
        modc_s[4 * D:5 * D, :] = modc_s[4 * D:5 * D, :] + 1.0
        prep_wo()
        d_w1.wait()
        d_w2.wait()
        attn((NB - 1) * TB, (NB - 1) % 2)
        for b in range(NB // 2):
            oproj(b * TB)
            prep_w1(b, NB // 2)
        for b in range(NB // 2, NB):
            oproj(b * TB)
            prep_w2(b - NB // 2, NB // 2)
            if b == NB // 2:
                ln2(0)

    def out_copy(b, slot):
        return pltpu.make_async_copy(out_s.at[slot], outT_hbm.at[:, _ds(b * TF, TF)], osems.at[slot])

    with _scope("s_floop"):
        @pl.loop(0, NF)
        def _(i):
            slot = i % 2

            @pl.when(i >= 2)
            def _():
                out_copy(i - 2, slot).wait()
            ffn(i, slot)
            ln2(jnp.minimum(i + 1, NF - 1))
            out_copy(i, slot).start()

    out_copy(NF - 2, NF % 2).wait()
    out_copy(NF - 1, (NF - 1) % 2).wait()


@jax.jit
def pallas_adaLN_cond__sliding_local_dilated__dense_activation_relu__prompt_kernel(
        A_x, A_wqkv, A_wo, B_x, B_w1, B_w2, c, w_mod):
    xT = A_x.reshape(S, D).T
    w2T = B_w2.T
    hbm = pl.BlockSpec(memory_space=pltpu.HBM)
    VM = pltpu.VMEM
    outT = pl.pallas_call(
        _kernel,
        in_specs=[hbm] * 7,
        out_specs=hbm,
        out_shape=jax.ShapeDtypeStruct((D, S), bf16),
        scratch_shapes=[
            VM((D, S), bf16),
            VM((D, 3 * D), bf16),
            VM((D, D), bf16),
            VM((D // 2, DFF), u32),
            VM((D // 2, DFF), u32),
            VM((1, D), bf16),
            VM((D, 6 * D), bf16),
            VM((5, 896, 128), u32),
            VM((3 * D // 2, D), u32),
            VM((D // 2, D), u32),
            VM((6 * D, 128), f32),
            VM((D, TB), bf16), VM((D, TB), bf16),
            VM((3 * D // 2, 128 + TB), u32), VM((3 * D // 2, 128 + TB), u32),
            VM((D // 2, S), u32),
            VM((D, S), f32),
            VM((NF * 7 * 64, 256), u32),
            VM((S // 2, 128), u32),
            VM((7 * 64, HF), u32),
            VM((5 * 128, HF), u32),
            VM((5 * 144, HF), u32),
            VM((2, D, TF), bf16),
            pltpu.SemaphoreType.DMA((9,)),
            pltpu.SemaphoreType.DMA((2,)),
        ],
        compiler_params=pltpu.CompilerParams(vmem_limit_bytes=110 * 1024 * 1024),
        name="adaln_attn_ffn_kernel",
    )(xT, A_wqkv, A_wo, B_w1, w2T, c, w_mod)
    return outT.T.reshape(1, S, D)
```

```python
import jax
import jax.numpy as jnp
from jax import lax
import jax.experimental.pallas as pl
import jax.experimental.pallas.tpu as pltpu

S, D, H, DH, W, DIL, DFF = 2048, 576, 32, 18, 8, 2, 4608
TB = 256
NB = S // TB
TF = 256
NF = S // TF
HF = DFF // 2
NJ = DH // 2
SCALE = float(DH ** -0.5)
EPS = 1e-5
LOG2E = 1.4426950408889634
NEG = -1e9
f32, bf16, u32, i32 = jnp.float32, jnp.bfloat16, jnp.uint32, jnp.int32
RSTEP = 8


def _ds(start, size, mult=128):
    if isinstance(start, int):
        return pl.ds(start, size)
    return pl.ds(pl.multiple_of(start, mult), size)


def _unp(x, i):
    return pltpu.unpack_elementwise(x, index=i, packed_dtype=bf16, unpacked_dtype=f32)


def _pk(a, b):
    return pltpu.pack_elementwise([a, b], packed_dtype=bf16)


def _ln(xf, a, b):
    m = jnp.sum(xf, axis=0, keepdims=True) * (1.0 / D)
    xc = xf - m
    v = jnp.sum(xc * xc, axis=0, keepdims=True) * (1.0 / D)
    return xc * lax.rsqrt(v + EPS) * a + b


def _kernel(xT_hbm, wqkv_hbm, wo_hbm, w1_hbm, w2T_hbm, c_hbm, wm_hbm, outT_hbm,
            x_s, wqkv_s, wo_s, w1_s, w2T_s, c_s, wm_s, tmp_s, wqT_s, woT_s, modc_s,
            hT_s, qb0, qb1, qb2, o_s, x1_s, xo_s, xr_s, hb_s, w1c_s, w2c_s, out_s, sc_s, sems, osems):
    qb = (qb0, qb1, qb2)

    def cp(i, src, dst):
        return pltpu.make_async_copy(src, dst, sems.at[i])
    NM1 = 2 * D
    XA, XB = 2 * TB, 4 * TB
    d_c = cp(0, c_hbm, c_s)
    d_wm1 = cp(1, wm_hbm.at[:, 0:NM1], wm_s.at[:, 0:NM1])
    d_x0 = cp(2, xT_hbm.bitcast(u32).at[:, 0:TB], x_s.at[:, 0:TB])
    d_x0b = cp(12, xT_hbm.bitcast(u32).at[:, TB:XA], x_s.at[:, TB:XA])
    d_wq = cp(3, wqkv_hbm.at[:, 0:640], wqkv_s.at[:, 0:640])
    d_wk = cp(10, wqkv_hbm.at[:, 640:2 * D], wqkv_s.at[:, 640:2 * D])
    d_wv = cp(9, wqkv_hbm.at[:, 2 * D:3 * D], wqkv_s.at[:, 2 * D:3 * D])
    d_x1 = cp(4, xT_hbm.bitcast(u32).at[:, XA:XB], x_s.at[:, XA:XB])
    d_x2 = cp(11, xT_hbm.bitcast(u32).at[:, XB:S], x_s.at[:, XB:S])
    d_wm2 = cp(5, wm_hbm.at[:, NM1:6 * D], wm_s.at[:, NM1:6 * D])
    d_wo = cp(6, wo_hbm, wo_s)
    d_w1 = cp(7, w1_hbm.bitcast(u32), w1_s)
    d_w2 = cp(8, w2T_hbm.bitcast(u32), w2T_s)
    for d in (d_c, d_wm1, d_wq, d_x0, d_x0b, d_wk, d_wv, d_x1, d_x2, d_wm2, d_wo, d_w1, d_w2):
        d.start()

    lane = lax.broadcasted_iota(i32, (8, 128), 1)

    def compute_mod(lo, hi):
        cf = c_s[...].astype(f32)
        sc = (cf * jax.nn.sigmoid(cf)).astype(bf16)
        sc_s[...] = jnp.broadcast_to(sc, (16, D))
        sc16 = jnp.broadcast_to(sc, (16, D))
        mod = jnp.dot(sc16, wm_s[:, lo:hi], preferred_element_type=f32)
        row = mod[0:1, :]
        for n in range((hi - lo) // 128):
            blk = jnp.broadcast_to(row[:, n * 128:(n + 1) * 128], (128, 128))
            modc_s[lo + n * 128: lo + (n + 1) * 128, :] = blk.T

    def mod_half(hf):
        lo = pl.multiple_of((1 + hf) * NM1, NM1)
        sc16 = jnp.broadcast_to(sc_s[0:1, :], (16, D))
        mod = jnp.dot(sc16, wm_s[:, pl.ds(lo, NM1)], preferred_element_type=f32)
        row = mod[0:1, :]
        plus = jnp.where(hf == 1, 1.0, 0.0)
        ridx = lax.broadcasted_iota(i32, (128, 128), 0)
        for n in range(NM1 // 128):
            blk = jnp.broadcast_to(row[:, n * 128:(n + 1) * 128], (128, 128)).T
            if n * 128 < D:
                blk = blk + jnp.where(ridx + n * 128 < D, plus, 0.0)
            modc_s[pl.ds(pl.multiple_of(lo + n * 128, 128), 128), :] = blk

    def modv(k):
        return modc_s[k * D:(k + 1) * D, :]

    def ln1(blk):
        G = D // 16
        for cc in range(TB // 128):
            col = slice(blk * TB + cc * 128, blk * TB + (cc + 1) * 128)
            acc0 = acc1 = None
            for g in range(G):
                w = x_s[8 * g:8 * g + 8, col]
                lo, hi = _unp(w, 0), _unp(w, 1)
                acc0 = lo if acc0 is None else acc0 + lo
                acc1 = hi if acc1 is None else acc1 + hi
            m = jnp.sum(acc0 + acc1, axis=0, keepdims=True) * (1.0 / D)
            acc0 = acc1 = None
            for g in range(G):
                w = x_s[8 * g:8 * g + 8, col]
                lo, hi = _unp(w, 0) - m, _unp(w, 1) - m
                acc0 = lo * lo if acc0 is None else acc0 + lo * lo
                acc1 = hi * hi if acc1 is None else acc1 + hi * hi
            v = jnp.sum(acc0 + acc1, axis=0, keepdims=True) * (1.0 / D)
            rstd = lax.rsqrt(v + EPS)
            for g in range(G):
                w = x_s[8 * g:8 * g + 8, col]
                ys = []
                for e in range(2):
                    a = modc_s[pl.ds(D + 16 * g + e, 8, stride=2), :]
                    b = modc_s[pl.ds(16 * g + e, 8, stride=2), :]
                    ys.append((_unp(w, e) - m) * rstd * a + b)
                hT_s[8 * g:8 * g + 8, col] = _pk(ys[0], ys[1])

    def qproj(base, slot):
        wt = pltpu.bitcast(wqT_s[...], bf16)
        hv = pltpu.bitcast(hT_s[:, _ds(base, TB, TB)], bf16)
        r = jnp.dot(wt, hv, preferred_element_type=f32).astype(bf16)
        qb[slot][:, 128:128 + TB] = pltpu.bitcast(r, u32)
        qb[(slot + 1) % 3][288:864, 0:128] = qb[slot][288:864, TB:TB + 128]

    def attn_chunk(base, slot, cc, masked):
        qr = qb[slot]
        cur = pl.ds(128 + cc * 128, 128)
        prev = pl.ds(cc * 128, 128)
        for hg in range(4):
            acc = [None] * W
            for j in range(NJ):
                r = j * 32 + hg * 8
                qw = qr[r:r + 8, cur]
                q0, q1 = _unp(qw, 0), _unp(qw, 1)
                kc = qr[288 + r:288 + r + 8, cur]
                kp = qr[288 + r:288 + r + 8, prev]
                for w in range(W):
                    ks = kc if w == 0 else pltpu.roll(jnp.where(lane < 128 - DIL * w, kc, kp), DIL * w, axis=1)
                    p = q0 * _unp(ks, 0) + q1 * _unp(ks, 1)
                    acc[w] = p if acc[w] is None else acc[w] + p
            lg = acc
            if masked and cc == 0:
                pos = lane + (base + cc * 128)
                lg = [lg[0]] + [jnp.where(pos >= DIL * w, lg[w], NEG / SCALE) for w in range(1, W)]
            m = lg[0]
            for w in range(1, W):
                m = jnp.maximum(m, lg[w])
            e = [jnp.exp2((l - m) * (SCALE * LOG2E)) for l in lg]
            s = e[0]
            for w in range(1, W):
                s = s + e[w]
            rinv = 1.0 / s
            p = [x * rinv for x in e]
            for j in range(NJ):
                r = j * 32 + hg * 8
                vc = qr[576 + r:576 + r + 8, cur]
                vp = qr[576 + r:576 + r + 8, prev]
                o0 = o1 = None
                for w in range(W):
                    vs = vc if w == 0 else pltpu.roll(jnp.where(lane < 128 - DIL * w, vc, vp), DIL * w, axis=1)
                    t0 = p[w] * _unp(vs, 0)
                    t1 = p[w] * _unp(vs, 1)
                    o0 = t0 if o0 is None else o0 + t0
                    o1 = t1 if o1 is None else o1 + t1
                o_s[r:r + 8, _ds(base + cc * 128, 128)] = _pk(o0, o1)

    def attn(base, slot, masked=False):
        for cc in range(TB // 128):
            attn_chunk(base, slot, cc, masked)

    def oproj2(base):
        wt = pltpu.bitcast(woT_s[...], bf16)
        ov = pltpu.bitcast(o_s[:, _ds(base, 2 * TB)], bf16)
        att = jnp.dot(wt, ov, preferred_element_type=f32)
        ga = modv(2)
        for cc in range(2 * TB // 128):
            c1 = _ds(base + cc * 128, 128)
            x1_s[:, c1] = pltpu.bitcast(x_s[:, c1], bf16).astype(f32) + ga * att[:, cc * 128:(cc + 1) * 128]

    def bc(v):
        return pltpu.bitcast(v, bf16)

    def ln2(blk):
        base = blk * TF
        hh = [_ln(x1_s[:, _ds(base + cc * 128, 128)], modv(4), modv(3)) for cc in range(2)]
        x11, x12, x21, x22 = hh[0][0:256], hh[0][256:512], hh[1][0:256], hh[1][256:512]
        ops = (x11 + x22, x21 + x22, x11, x22, x11 + x12, x21 - x11, x12 - x22)
        for k in range(7):
            xo_s[_ds(blk * 448 + k * 64, 64, 64), :] = pltpu.bitcast(ops[k].astype(bf16).T, u32)
        for cc in range(2):
            xr_s[_ds(blk * 128 + cc * 64, 64, 64), 0:64] = pltpu.bitcast(hh[cc][512:D].astype(bf16).T, u32)

    def ffn(blk, slot):
        base = blk * TF
        TN = 128
        xs = [bc(xo_s[_ds(blk * 448 + k * 64, 64, 64), :]) for k in range(7)]
        xr = bc(xr_s[_ds(blk * 128, 128, 128), :])[:, 0:64]
        for j in range(HF // TN):
            c1 = slice(j * TN, (j + 1) * TN)
            c2 = slice(HF + j * TN, HF + (j + 1) * TN)
            wk = (w1c_s[0:128, c1], w1_s[0:128, c1], w1c_s[128:256, c1], w1c_s[256:384, c1],
                  w1_s[128:256, c2], w1c_s[384:512, c1], w1c_s[512:640, c1])
            r1 = jnp.dot(xr, bc(w1_s[256:288, c1]), preferred_element_type=f32)
            r2 = jnp.dot(xr, bc(w1_s[256:288, c2]), preferred_element_type=f32)
            m = [jnp.dot(xs[k], bc(wk[k]), preferred_element_type=f32) for k in range(7)]
            h11 = m[0] + m[3] - m[4] + m[6] + r1[0:128]
            h12 = m[2] + m[4] + r2[0:128]
            h21 = m[1] + m[3] + r1[128:256]
            h22 = m[0] - m[1] + m[2] + m[5] + r2[128:256]
            b11 = jnp.maximum(h11, 0.0)
            b12 = jnp.maximum(h21, 0.0)
            b21 = jnp.maximum(h12, 0.0)
            b22 = jnp.maximum(h22, 0.0)
            bs = (b11 + b22, b11, b12 - b22, b21 - b11, b22, b11 + b12, b21 + b22)
            for k in range(7):
                hb_s[k * 64:(k + 1) * 64, c1] = pltpu.bitcast(bs[k].astype(bf16), u32)
        ak = (w2c_s[0:144, :], w2c_s[144:288, :], w2T_s[0:144, 0:HF], w2T_s[144:288, HF:DFF],
              w2c_s[288:432, :], w2c_s[432:576, :], w2c_s[576:720, :])
        m = [lax.dot_general(bc(ak[k]), bc(hb_s[k * 64:(k + 1) * 64, :]), (((1,), (1,)), ((), ())),
                             preferred_element_type=f32) for k in range(7)]
        cq = ((m[0] + m[3] - m[4] + m[6], m[2] + m[4]), (m[1] + m[3], m[0] - m[1] + m[2] + m[5]))
        for r in range(2):
            rr = slice(r * 288, (r + 1) * 288)
            gb = modc_s[5 * D + r * 288:5 * D + (r + 1) * 288, :]
            for cc in range(2):
                c1 = _ds(base + cc * 128, 128)
                out_s[slot, rr, cc * 128:(cc + 1) * 128] = (x1_s[rr, c1] + gb * cq[r][cc]).astype(bf16)

    def combos(dst, src, rows, signs2):
        for cidx in range(HF // 128):
            c1 = slice(cidx * 128, (cidx + 1) * 128)
            c2 = slice(HF + cidx * 128, HF + (cidx + 1) * 128)
            for r0 in range(0, rows, RSTEP):
                ra = slice(r0, r0 + RSTEP)
                rb = slice(rows + r0, rows + r0 + RSTEP)
                quad = [src[ra, c1], src[ra, c2], src[rb, c1], src[rb, c2]]
                lo = [_unp(q, 0) for q in quad]
                hi = [_unp(q, 1) for q in quad]
                for n, (ia, ib, sgn) in enumerate(signs2):
                    rd = slice(n * rows + r0, n * rows + r0 + RSTEP)
                    if sgn > 0:
                        dst[rd, c1] = _pk(lo[ia] + lo[ib], hi[ia] + hi[ib])
                    else:
                        dst[rd, c1] = _pk(lo[ia] - lo[ib], hi[ia] - hi[ib])

    def prep_w1():
        combos(w1c_s, w1_s, 128, ((0, 3, 1), (1, 3, -1), (2, 0, -1), (0, 1, 1), (2, 3, 1)))

    def prep_w2():
        combos(w2c_s, w2T_s, 144, ((0, 3, 1), (2, 3, 1), (0, 1, 1), (2, 0, -1), (1, 3, -1)))

    def prep_wqkv(c0, c1, w0, w1):
        for cidx in range(c0, c1):
            ncol = 128 if cidx < 13 else 64
            t = wqkv_s[:, cidx * 128: cidx * 128 + ncol].T
            tw = pltpu.bitcast(t, u32)
            for kt in range(5):
                kw = 128 if kt < 4 else 64
                tmp_s[kt, cidx * 64: cidx * 64 + ncol // 2, 0:kw] = tw[:, kt * 128: kt * 128 + kw]
        for which in range(w0, w1):
            for j in range(NJ):
                for kt in range(5):
                    kw = 128 if kt < 4 else 64
                    v = tmp_s[kt, pl.ds(which * 288 + j, 32, stride=NJ), :]
                    wqT_s[which * 288 + j * 32: which * 288 + (j + 1) * 32, kt * 128: kt * 128 + kw] = v[:, 0:kw]

    def prep_wo():
        wv = pltpu.bitcast(wo_s[...], u32)
        for nt in range(5):
            nw = 128 if nt < 4 else 64
            tmp_s[nt, 0:288, 0:nw] = wv[:, nt * 128: nt * 128 + nw]
        for nt in range(5):
            nw = 128 if nt < 4 else 64
            parts = [tmp_s[nt, pl.ds(j, 32, stride=NJ), :] for j in range(NJ)]
            pw = jnp.concatenate(parts, axis=0)
            pb = pltpu.bitcast(pw, bf16)
            tt = pb[:, 0:nw].T
            woT_s[nt * 64: nt * 64 + nw // 2, :] = pltpu.bitcast(tt, u32)

    qb0[288:864, 0:128] = jnp.zeros((576, 128), u32)
    d_c.wait()
    d_wm1.wait()
    compute_mod(0, NM1)
    modc_s[D:2 * D, :] = modc_s[D:2 * D, :] + 1.0
    d_wq.wait()
    prep_wqkv(0, 5, 0, 1)
    d_x0.wait()
    ln1(0)
    d_x0b.wait()
    ln1(1)

    def qpart(r0, r1):
        wt = pltpu.bitcast(wqT_s[r0:r1, :], bf16)
        hv = pltpu.bitcast(hT_s[:, 0:2 * TB], bf16)
        r = pltpu.bitcast(jnp.dot(wt, hv, preferred_element_type=f32).astype(bf16), u32)
        qb0[r0:r1, 128:128 + TB] = r[:, 0:TB]
        qb1[r0:r1, 128:128 + TB] = r[:, TB:2 * TB]
        if r0 >= 288:
            qb1[r0:r1, 0:128] = qb0[r0:r1, TB:TB + 128]

    qpart(0, 144)
    d_wk.wait()
    qpart(144, 288)
    prep_wqkv(5, 9, 1, 2)
    d_wv.wait()
    d_x1.wait()
    qpart(288, 576)
    prep_wqkv(9, 14, 2, 3)
    ln1(2)
    ln1(3)
    d_x2.wait()
    qpart(576, 864)
    for blk in range(4, NB):
        ln1(blk)
    qb2[288:864, 0:128] = qb1[288:864, TB:TB + 128]

    def body(i, slot, masked=False):
        attn((i - 2) * TB, (slot + 1) % 3, masked)
        qproj(i * TB, slot)

    d_wm2.wait()

    @pl.loop(0, (NB - 2) // 3)
    def _(ii):
        i = 2 + 3 * ii
        mod_half(ii)
        body(i, 2, True)
        body(i + 1, 0)
        body(i + 2, 1)

    d_wo.wait()
    prep_wo()
    attn((NB - 2) * TB, (NB - 2) % 3)
    attn((NB - 1) * TB, (NB - 1) % 3)
    oproj2(0)
    oproj2(2 * TB)
    oproj2(4 * TB)
    d_w1.wait()
    d_w2.wait()
    prep_w1()
    prep_w2()
    oproj2(6 * TB)
    ln2(0)

    def out_copy(b, slot):
        return pltpu.make_async_copy(out_s.at[slot], outT_hbm.at[:, _ds(b * TF, TF)], osems.at[slot])

    @pl.loop(0, NF)
    def _(i):
        slot = i % 2

        @pl.when(i >= 2)
        def _():
            out_copy(i - 2, slot).wait()
        ffn(i, slot)
        ln2(jnp.minimum(i + 1, NF - 1))
        out_copy(i, slot).start()

    out_copy(NF - 2, NF % 2).wait()
    out_copy(NF - 1, (NF - 1) % 2).wait()


@jax.jit
def pallas_adaLN_cond__sliding_local_dilated__dense_activation_relu__prompt_kernel(
        A_x, A_wqkv, A_wo, B_x, B_w1, B_w2, c, w_mod):
    xT = A_x.reshape(S, D).T
    w2T = B_w2.T
    hbm = pl.BlockSpec(memory_space=pltpu.HBM)
    VM = pltpu.VMEM
    outT = pl.pallas_call(
        _kernel,
        in_specs=[hbm] * 7,
        out_specs=hbm,
        out_shape=jax.ShapeDtypeStruct((D, S), bf16),
        scratch_shapes=[
            VM((D // 2, S), u32),
            VM((D, 3 * D), bf16),
            VM((D, D), bf16),
            VM((D // 2, DFF), u32),
            VM((D // 2, DFF), u32),
            VM((1, D), bf16),
            VM((D, 6 * D), bf16),
            VM((5, 896, 128), u32),
            VM((3 * D // 2, D), u32),
            VM((D // 2, D), u32),
            VM((6 * D, 128), f32),
            VM((D // 2, S), u32),
            VM((3 * D // 2, 128 + TB), u32), VM((3 * D // 2, 128 + TB), u32),
            VM((3 * D // 2, 128 + TB), u32),
            VM((D // 2, S), u32),
            VM((D, S), f32),
            VM((NF * 7 * 64, 256), u32),
            VM((S // 2, 128), u32),
            VM((7 * 64, HF), u32),
            VM((5 * 128, HF), u32),
            VM((5 * 144, HF), u32),
            VM((2, D, TF), bf16),
            VM((16, D), bf16),
            pltpu.SemaphoreType.DMA((13,)),
            pltpu.SemaphoreType.DMA((2,)),
        ],
        compiler_params=pltpu.CompilerParams(vmem_limit_bytes=110 * 1024 * 1024, flags={'XLA_TPU_EVENLY_DISTRIBUTE_CRITICAL_NODES': True}),
        name="adaln_attn_ffn_kernel",
    )(xT, A_wqkv, A_wo, B_w1, w2T, c, w_mod)
    return outT.T.reshape(1, S, D)
```

```python
import jax
import jax.numpy as jnp
from jax import lax
import jax.experimental.pallas as pl
import jax.experimental.pallas.tpu as pltpu

S, D, H, DH, W, DIL, DFF = 2048, 576, 32, 18, 8, 2, 4608
TB = 256
NB = S // TB
TF = 256
NF = S // TF
HF = DFF // 2
NJ = DH // 2
SCALE = float(DH ** -0.5)
EPS = 1e-5
LOG2E = 1.4426950408889634
NEG = -1e9
f32, bf16, u32, i32 = jnp.float32, jnp.bfloat16, jnp.uint32, jnp.int32
RSTEP = 8


def _ds(start, size, mult=128):
    if isinstance(start, int):
        return pl.ds(start, size)
    return pl.ds(pl.multiple_of(start, mult), size)


def _unp(x, i):
    return pltpu.unpack_elementwise(x, index=i, packed_dtype=bf16, unpacked_dtype=f32)


def _pk(a, b):
    return pltpu.pack_elementwise([a, b], packed_dtype=bf16)


def _ln(xf, a, b):
    m = jnp.sum(xf, axis=0, keepdims=True) * (1.0 / D)
    xc = xf - m
    v = jnp.sum(xc * xc, axis=0, keepdims=True) * (1.0 / D)
    return xc * lax.rsqrt(v + EPS) * a + b


def _kernel(xT_hbm, wqkv_hbm, wo_hbm, w1_hbm, w2T_hbm, c_hbm, wm_hbm, outT_hbm,
            x_s, wqkv_s, wo_s, w1_s, w2T_s, c_s, wm_s, tmp_s, wqT_s, woT_s, modc_s,
            hT_s, qb0, qb1, qb2, o_s, x1_s, xo_s, xr_s, hb_s, w1c_s, w2c_s, out_s, sc_s, sems, osems, wsems):
    qb = (qb0, qb1, qb2)

    def cp(i, src, dst):
        return pltpu.make_async_copy(src, dst, sems.at[i])
    NM1 = 2 * D
    XA, XB = 2 * TB, 4 * TB
    d_c = cp(0, c_hbm, c_s)
    d_wm1 = cp(1, wm_hbm.at[:, 0:NM1], wm_s.at[:, 0:NM1])
    d_x0 = cp(2, xT_hbm.bitcast(u32).at[:, 0:TB], x_s.at[:, 0:TB])
    d_x0b = cp(12, xT_hbm.bitcast(u32).at[:, TB:XA], x_s.at[:, TB:XA])
    d_wq = cp(3, wqkv_hbm.at[:, 0:640], wqkv_s.at[:, 0:640])
    d_wk = cp(10, wqkv_hbm.at[:, 640:2 * D], wqkv_s.at[:, 640:2 * D])
    d_wv = cp(9, wqkv_hbm.at[:, 2 * D:3 * D], wqkv_s.at[:, 2 * D:3 * D])
    d_x1 = cp(4, xT_hbm.bitcast(u32).at[:, XA:XB], x_s.at[:, XA:XB])
    d_x2 = cp(11, xT_hbm.bitcast(u32).at[:, XB:S], x_s.at[:, XB:S])
    d_wm2 = cp(5, wm_hbm.at[:, NM1:6 * D], wm_s.at[:, NM1:6 * D])
    d_wo = cp(6, wo_hbm, wo_s)
    HQ = HF // 2

    def d_w1(hf, part):
        cols = _ds(part * HF + hf * HQ, HQ, HQ)
        return pltpu.make_async_copy(w1_hbm.bitcast(u32).at[:, cols], w1_s.at[:, cols], wsems.at[hf * 2 + part])
    d_w2 = cp(8, w2T_hbm.bitcast(u32), w2T_s)
    for d in (d_c, d_wm1, d_wq, d_x0, d_x0b, d_wk, d_wv, d_x1, d_x2, d_wm2, d_w1(0, 0), d_w1(0, 1), d_w1(1, 0), d_w1(1, 1), d_wo, d_w2):
        d.start()

    lane = lax.broadcasted_iota(i32, (8, 128), 1)

    def compute_mod(lo, hi):
        cf = c_s[...].astype(f32)
        sc = (cf * jax.nn.sigmoid(cf)).astype(bf16)
        sc_s[...] = jnp.broadcast_to(sc, (16, D))
        sc16 = jnp.broadcast_to(sc, (16, D))
        mod = jnp.dot(sc16, wm_s[:, lo:hi], preferred_element_type=f32)
        row = mod[0:1, :]
        for n in range((hi - lo) // 128):
            blk = jnp.broadcast_to(row[:, n * 128:(n + 1) * 128], (128, 128))
            modc_s[lo + n * 128: lo + (n + 1) * 128, :] = blk.T

    def mod_half(hf):
        lo = pl.multiple_of((1 + hf) * NM1, NM1)
        sc16 = jnp.broadcast_to(sc_s[0:1, :], (16, D))
        mod = jnp.dot(sc16, wm_s[:, pl.ds(lo, NM1)], preferred_element_type=f32)
        row = mod[0:1, :]
        plus = jnp.where(hf == 1, 1.0, 0.0)
        ridx = lax.broadcasted_iota(i32, (128, 128), 0)
        for n in range(NM1 // 128):
            blk = jnp.broadcast_to(row[:, n * 128:(n + 1) * 128], (128, 128)).T
            if n * 128 < D:
                blk = blk + jnp.where(ridx + n * 128 < D, plus, 0.0)
            modc_s[pl.ds(pl.multiple_of(lo + n * 128, 128), 128), :] = blk

    def modv(k):
        return modc_s[k * D:(k + 1) * D, :]

    def ln1(blk):
        G = D // 16
        for cc in range(TB // 128):
            col = slice(blk * TB + cc * 128, blk * TB + (cc + 1) * 128)
            acc0 = acc1 = None
            for g in range(G):
                w = x_s[8 * g:8 * g + 8, col]
                lo, hi = _unp(w, 0), _unp(w, 1)
                acc0 = lo if acc0 is None else acc0 + lo
                acc1 = hi if acc1 is None else acc1 + hi
            m = jnp.sum(acc0 + acc1, axis=0, keepdims=True) * (1.0 / D)
            acc0 = acc1 = None
            for g in range(G):
                w = x_s[8 * g:8 * g + 8, col]
                lo, hi = _unp(w, 0) - m, _unp(w, 1) - m
                acc0 = lo * lo if acc0 is None else acc0 + lo * lo
                acc1 = hi * hi if acc1 is None else acc1 + hi * hi
            v = jnp.sum(acc0 + acc1, axis=0, keepdims=True) * (1.0 / D)
            rstd = lax.rsqrt(v + EPS)
            for g in range(G):
                w = x_s[8 * g:8 * g + 8, col]
                ys = []
                for e in range(2):
                    a = modc_s[pl.ds(D + 16 * g + e, 8, stride=2), :]
                    b = modc_s[pl.ds(16 * g + e, 8, stride=2), :]
                    ys.append((_unp(w, e) - m) * rstd * a + b)
                hT_s[8 * g:8 * g + 8, col] = _pk(ys[0], ys[1])

    def qproj(base, slot):
        wt = pltpu.bitcast(wqT_s[...], bf16)
        hv = pltpu.bitcast(hT_s[:, _ds(base, TB, TB)], bf16)
        r = jnp.dot(wt, hv, preferred_element_type=f32).astype(bf16)
        qb[slot][:, 128:128 + TB] = pltpu.bitcast(r, u32)
        qb[(slot + 1) % 3][288:864, 0:128] = qb[slot][288:864, TB:TB + 128]

    def attn_chunk(base, slot, cc, masked):
        qr = qb[slot]
        cur = pl.ds(128 + cc * 128, 128)
        prev = pl.ds(cc * 128, 128)
        for hg in range(4):
            acc = [None] * W
            for j in range(NJ):
                r = j * 32 + hg * 8
                qw = qr[r:r + 8, cur]
                q0, q1 = _unp(qw, 0), _unp(qw, 1)
                kc = qr[288 + r:288 + r + 8, cur]
                kp = qr[288 + r:288 + r + 8, prev]
                for w in range(W):
                    ks = kc if w == 0 else pltpu.roll(jnp.where(lane < 128 - DIL * w, kc, kp), DIL * w, axis=1)
                    p = q0 * _unp(ks, 0) + q1 * _unp(ks, 1)
                    acc[w] = p if acc[w] is None else acc[w] + p
            lg = acc
            if masked and cc == 0:
                pos = lane + (base + cc * 128)
                lg = [lg[0]] + [jnp.where(pos >= DIL * w, lg[w], NEG / SCALE) for w in range(1, W)]
            m = lg[0]
            for w in range(1, W):
                m = jnp.maximum(m, lg[w])
            e = [jnp.exp2((l - m) * (SCALE * LOG2E)) for l in lg]
            s = e[0]
            for w in range(1, W):
                s = s + e[w]
            rinv = 1.0 / s
            p = [x * rinv for x in e]
            for j in range(NJ):
                r = j * 32 + hg * 8
                vc = qr[576 + r:576 + r + 8, cur]
                vp = qr[576 + r:576 + r + 8, prev]
                o0 = o1 = None
                for w in range(W):
                    vs = vc if w == 0 else pltpu.roll(jnp.where(lane < 128 - DIL * w, vc, vp), DIL * w, axis=1)
                    t0 = p[w] * _unp(vs, 0)
                    t1 = p[w] * _unp(vs, 1)
                    o0 = t0 if o0 is None else o0 + t0
                    o1 = t1 if o1 is None else o1 + t1
                o_s[r:r + 8, _ds(base + cc * 128, 128)] = _pk(o0, o1)

    def attn(base, slot, masked=False):
        for cc in range(TB // 128):
            attn_chunk(base, slot, cc, masked)

    def oproj2(base):
        wt = pltpu.bitcast(woT_s[...], bf16)
        ov = pltpu.bitcast(o_s[:, _ds(base, 2 * TB)], bf16)
        att = jnp.dot(wt, ov, preferred_element_type=f32)
        ga = modv(2)
        for cc in range(2 * TB // 128):
            c1 = _ds(base + cc * 128, 128)
            x1_s[:, c1] = pltpu.bitcast(x_s[:, c1], bf16).astype(f32) + ga * att[:, cc * 128:(cc + 1) * 128]

    def bc(v):
        return pltpu.bitcast(v, bf16)

    def ln2(blk):
        base = blk * TF
        hh = [_ln(x1_s[:, _ds(base + cc * 128, 128)], modv(4), modv(3)) for cc in range(2)]
        x11, x12, x21, x22 = hh[0][0:256], hh[0][256:512], hh[1][0:256], hh[1][256:512]
        ops = (x11 + x22, x21 + x22, x11, x22, x11 + x12, x21 - x11, x12 - x22)
        for k in range(7):
            xo_s[_ds(blk * 448 + k * 64, 64, 64), :] = pltpu.bitcast(ops[k].astype(bf16).T, u32)
        for cc in range(2):
            xr_s[_ds(blk * 128 + cc * 64, 64, 64), 0:64] = pltpu.bitcast(hh[cc][512:D].astype(bf16).T, u32)

    def ffn(blk, slot):
        base = blk * TF
        TN = 128
        xs = [bc(xo_s[_ds(blk * 448 + k * 64, 64, 64), :]) for k in range(7)]
        xr = bc(xr_s[_ds(blk * 128, 128, 128), :])[:, 0:64]
        for j in range(HF // TN):
            c1 = slice(j * TN, (j + 1) * TN)
            c2 = slice(HF + j * TN, HF + (j + 1) * TN)
            wk = (w1c_s[0:128, c1], w1_s[0:128, c1], w1c_s[128:256, c1], w1c_s[256:384, c1],
                  w1_s[128:256, c2], w1c_s[384:512, c1], w1c_s[512:640, c1])
            r1 = jnp.dot(xr, bc(w1_s[256:288, c1]), preferred_element_type=f32)
            r2 = jnp.dot(xr, bc(w1_s[256:288, c2]), preferred_element_type=f32)
            m = [jnp.dot(xs[k], bc(wk[k]), preferred_element_type=f32) for k in range(7)]
            h11 = m[0] + m[3] - m[4] + m[6] + r1[0:128]
            h12 = m[2] + m[4] + r2[0:128]
            h21 = m[1] + m[3] + r1[128:256]
            h22 = m[0] - m[1] + m[2] + m[5] + r2[128:256]
            b11 = jnp.maximum(h11, 0.0)
            b12 = jnp.maximum(h21, 0.0)
            b21 = jnp.maximum(h12, 0.0)
            b22 = jnp.maximum(h22, 0.0)
            bs = (b11 + b22, b11, b12 - b22, b21 - b11, b22, b11 + b12, b21 + b22)
            for k in range(7):
                hb_s[k * 64:(k + 1) * 64, c1] = pltpu.bitcast(bs[k].astype(bf16), u32)
        ak = (w2c_s[0:144, :], w2c_s[144:288, :], w2T_s[0:144, 0:HF], w2T_s[144:288, HF:DFF],
              w2c_s[288:432, :], w2c_s[432:576, :], w2c_s[576:720, :])
        m = [lax.dot_general(bc(ak[k]), bc(hb_s[k * 64:(k + 1) * 64, :]), (((1,), (1,)), ((), ())),
                             preferred_element_type=f32) for k in range(7)]
        cq = ((m[0] + m[3] - m[4] + m[6], m[2] + m[4]), (m[1] + m[3], m[0] - m[1] + m[2] + m[5]))
        for r in range(2):
            rr = slice(r * 288, (r + 1) * 288)
            gb = modc_s[5 * D + r * 288:5 * D + (r + 1) * 288, :]
            for cc in range(2):
                c1 = _ds(base + cc * 128, 128)
                out_s[slot, rr, cc * 128:(cc + 1) * 128] = (x1_s[rr, c1] + gb * cq[r][cc]).astype(bf16)

    def combos(dst, src, rows, signs2, c0=0, ncol=HF // 128):
        for cidx in range(ncol):
            c1 = _ds(c0 + cidx * 128, 128)
            c2 = _ds(HF + c0 + cidx * 128, 128)
            for r0 in range(0, rows, RSTEP):
                ra = slice(r0, r0 + RSTEP)
                rb = slice(rows + r0, rows + r0 + RSTEP)
                quad = [src[ra, c1], src[ra, c2], src[rb, c1], src[rb, c2]]
                lo = [_unp(q, 0) for q in quad]
                hi = [_unp(q, 1) for q in quad]
                for n, (ia, ib, sgn) in enumerate(signs2):
                    rd = slice(n * rows + r0, n * rows + r0 + RSTEP)
                    if sgn > 0:
                        dst[rd, c1] = _pk(lo[ia] + lo[ib], hi[ia] + hi[ib])
                    else:
                        dst[rd, c1] = _pk(lo[ia] - lo[ib], hi[ia] - hi[ib])

    def prep_w1(hf):
        combos(w1c_s, w1_s, 128, ((0, 3, 1), (1, 3, -1), (2, 0, -1), (0, 1, 1), (2, 3, 1)), hf * HQ, HQ // 128)

    def prep_w2():
        combos(w2c_s, w2T_s, 144, ((0, 3, 1), (2, 3, 1), (0, 1, 1), (2, 0, -1), (1, 3, -1)))

    def prep_wqkv(c0, c1, w0, w1):
        for cidx in range(c0, c1):
            ncol = 128 if cidx < 13 else 64
            t = wqkv_s[:, cidx * 128: cidx * 128 + ncol].T
            tw = pltpu.bitcast(t, u32)
            for kt in range(5):
                kw = 128 if kt < 4 else 64
                tmp_s[kt, cidx * 64: cidx * 64 + ncol // 2, 0:kw] = tw[:, kt * 128: kt * 128 + kw]
        for which in range(w0, w1):
            for j in range(NJ):
                for kt in range(5):
                    kw = 128 if kt < 4 else 64
                    v = tmp_s[kt, pl.ds(which * 288 + j, 32, stride=NJ), :]
                    wqT_s[which * 288 + j * 32: which * 288 + (j + 1) * 32, kt * 128: kt * 128 + kw] = v[:, 0:kw]

    def prep_wo():
        wv = pltpu.bitcast(wo_s[...], u32)
        for nt in range(5):
            nw = 128 if nt < 4 else 64
            tmp_s[nt, 0:288, 0:nw] = wv[:, nt * 128: nt * 128 + nw]
        for nt in range(5):
            nw = 128 if nt < 4 else 64
            parts = [tmp_s[nt, pl.ds(j, 32, stride=NJ), :] for j in range(NJ)]
            pw = jnp.concatenate(parts, axis=0)
            pb = pltpu.bitcast(pw, bf16)
            tt = pb[:, 0:nw].T
            woT_s[nt * 64: nt * 64 + nw // 2, :] = pltpu.bitcast(tt, u32)

    qb0[288:864, 0:128] = jnp.zeros((576, 128), u32)
    d_c.wait()
    d_wm1.wait()
    compute_mod(0, NM1)
    modc_s[D:2 * D, :] = modc_s[D:2 * D, :] + 1.0
    d_wq.wait()
    prep_wqkv(0, 5, 0, 1)
    d_x0.wait()
    ln1(0)
    d_x0b.wait()
    ln1(1)

    def qpart(r0, r1):
        wt = pltpu.bitcast(wqT_s[r0:r1, :], bf16)
        hv = pltpu.bitcast(hT_s[:, 0:2 * TB], bf16)
        r = pltpu.bitcast(jnp.dot(wt, hv, preferred_element_type=f32).astype(bf16), u32)
        qb0[r0:r1, 128:128 + TB] = r[:, 0:TB]
        qb1[r0:r1, 128:128 + TB] = r[:, TB:2 * TB]
        if r0 >= 288:
            qb1[r0:r1, 0:128] = qb0[r0:r1, TB:TB + 128]

    qpart(0, 144)
    d_wk.wait()
    qpart(144, 288)
    prep_wqkv(5, 9, 1, 2)
    d_wv.wait()
    d_x1.wait()
    qpart(288, 576)
    prep_wqkv(9, 14, 2, 3)
    ln1(2)
    ln1(3)
    d_x2.wait()
    qpart(576, 864)
    for blk in range(4, NB):
        ln1(blk)
    qb2[288:864, 0:128] = qb1[288:864, TB:TB + 128]

    def body(i, slot, masked=False):
        attn((i - 2) * TB, (slot + 1) % 3, masked)
        qproj(i * TB, slot)

    d_wm2.wait()

    @pl.loop(0, (NB - 2) // 3)
    def _(ii):
        i = 2 + 3 * ii
        mod_half(ii)
        body(i, 2, True)
        d_w1(ii, 0).wait()
        d_w1(ii, 1).wait()
        prep_w1(ii)
        body(i + 1, 0)
        body(i + 2, 1)

    d_wo.wait()
    prep_wo()
    attn((NB - 2) * TB, (NB - 2) % 3)
    attn((NB - 1) * TB, (NB - 1) % 3)
    oproj2(0)
    oproj2(2 * TB)
    oproj2(4 * TB)
    d_w2.wait()
    prep_w2()
    oproj2(6 * TB)
    ln2(0)

    def out_copy(b, slot):
        return pltpu.make_async_copy(out_s.at[slot], outT_hbm.at[:, _ds(b * TF, TF)], osems.at[slot])

    @pl.loop(0, NF)
    def _(i):
        slot = i % 2

        @pl.when(i >= 2)
        def _():
            out_copy(i - 2, slot).wait()
        ffn(i, slot)
        ln2(jnp.minimum(i + 1, NF - 1))
        out_copy(i, slot).start()

    out_copy(NF - 2, NF % 2).wait()
    out_copy(NF - 1, (NF - 1) % 2).wait()


@jax.jit
def pallas_adaLN_cond__sliding_local_dilated__dense_activation_relu__prompt_kernel(
        A_x, A_wqkv, A_wo, B_x, B_w1, B_w2, c, w_mod):
    xT = A_x.reshape(S, D).T
    w2T = B_w2.T
    hbm = pl.BlockSpec(memory_space=pltpu.HBM)
    VM = pltpu.VMEM
    outT = pl.pallas_call(
        _kernel,
        in_specs=[hbm] * 7,
        out_specs=hbm,
        out_shape=jax.ShapeDtypeStruct((D, S), bf16),
        scratch_shapes=[
            VM((D // 2, S), u32),
            VM((D, 3 * D), bf16),
            VM((D, D), bf16),
            VM((D // 2, DFF), u32),
            VM((D // 2, DFF), u32),
            VM((1, D), bf16),
            VM((D, 6 * D), bf16),
            VM((5, 896, 128), u32),
            VM((3 * D // 2, D), u32),
            VM((D // 2, D), u32),
            VM((6 * D, 128), f32),
            VM((D // 2, S), u32),
            VM((3 * D // 2, 128 + TB), u32), VM((3 * D // 2, 128 + TB), u32),
            VM((3 * D // 2, 128 + TB), u32),
            VM((D // 2, S), u32),
            VM((D, S), f32),
            VM((NF * 7 * 64, 256), u32),
            VM((S // 2, 128), u32),
            VM((7 * 64, HF), u32),
            VM((5 * 128, HF), u32),
            VM((5 * 144, HF), u32),
            VM((2, D, TF), bf16),
            VM((16, D), bf16),
            pltpu.SemaphoreType.DMA((13,)),
            pltpu.SemaphoreType.DMA((2,)),
            pltpu.SemaphoreType.DMA((4,)),
        ],
        compiler_params=pltpu.CompilerParams(vmem_limit_bytes=110 * 1024 * 1024, flags={'XLA_TPU_EVENLY_DISTRIBUTE_CRITICAL_NODES': True}),
        name="adaln_attn_ffn_kernel",
    )(xT, A_wqkv, A_wo, B_w1, w2T, c, w_mod)
    return outT.T.reshape(1, S, D)
```

```python
import jax
import jax.numpy as jnp
import numpy as np
from jax import lax
import jax.experimental.pallas as pl
import jax.experimental.pallas.tpu as pltpu

S, D, DH, W, DIL, DFF = 2048, 576, 18, 8, 2, 4608
TB = 256
NB = S // TB
TF = 256
NF = S // TF
HF = DFF // 2
NJ = DH // 2
SCALE = float(DH ** -0.5)
EPS = 1e-5
LOG2E = 1.4426950408889634
NEG = -1e9
f32, bf16, u32, i32 = jnp.float32, jnp.bfloat16, jnp.uint32, jnp.int32
RSTEP = 8


def _ds(start, size, mult=128):
    if isinstance(start, int):
        return pl.ds(start, size)
    return pl.ds(pl.multiple_of(start, mult), size)


def _unp(x, i):
    return pltpu.bitcast((x << 16) if i == 0 else (x & np.uint32(0xFFFF0000)), f32)


def _f32(words):
    return pltpu.bitcast(words, bf16).astype(f32)


def _words(rows):
    return pltpu.bitcast(rows.astype(bf16), u32)


def _ln(xf, a, b):
    m = jnp.sum(xf, axis=0, keepdims=True) * (1.0 / D)
    xc = xf - m
    v = jnp.sum(xc * xc, axis=0, keepdims=True) * (1.0 / D)
    return xc * lax.rsqrt(v + EPS) * a + b


def _kernel(xT_hbm, wqkv_hbm, wo_hbm, w1_hbm, w2T_hbm, c_hbm, wm_hbm, outT_hbm,
            x_s, wqkv_s, wo_s, w1_s, w2T_s, c_s, wm_s, tmp_s, wqT_s, woT_s, modc_s,
            hT_s, qb0, qb1, qb2, o_s, x1_s, xo_s, xr_s, hb_s, w1c_s, w2c_s, out_s, sc_s, wof_s, sems, osems, wsems):
    qb = (qb0, qb1, qb2)

    def cp(i, src, dst):
        return pltpu.make_async_copy(src, dst, sems.at[i])
    NM1 = 2 * D
    XA, XB = 2 * TB, 4 * TB
    d_c = cp(0, c_hbm, c_s)
    d_wm1 = cp(1, wm_hbm.at[:, 0:NM1], wm_s.at[:, 0:NM1])
    d_x0 = cp(2, xT_hbm.bitcast(u32).at[:, 0:TB], x_s.at[:, 0:TB])
    d_x0b = cp(12, xT_hbm.bitcast(u32).at[:, TB:XA], x_s.at[:, TB:XA])
    d_wq = cp(3, wqkv_hbm.at[:, 0:640], wqkv_s.at[:, 0:640])
    d_wk = cp(10, wqkv_hbm.at[:, 640:2 * D], wqkv_s.at[:, 640:2 * D])
    d_wv = cp(9, wqkv_hbm.at[:, 2 * D:3 * D], wqkv_s.at[:, 2 * D:3 * D])
    d_x1 = cp(4, xT_hbm.bitcast(u32).at[:, XA:XB], x_s.at[:, XA:XB])
    d_x2 = cp(11, xT_hbm.bitcast(u32).at[:, XB:S], x_s.at[:, XB:S])
    d_wm2 = cp(5, wm_hbm.at[:, NM1:6 * D], wm_s.at[:, NM1:6 * D])
    d_wo = cp(6, wo_hbm, wo_s)
    HQ = HF // 2

    def d_w1(hf, part):
        cols = _ds(part * HF + hf * HQ, HQ, HQ)
        return pltpu.make_async_copy(w1_hbm.bitcast(u32).at[:, cols], w1_s.at[:, cols], wsems.at[hf * 2 + part])

    d_w2 = cp(8, w2T_hbm.bitcast(u32), w2T_s)
    for d in (d_c, d_wm1, d_wq, d_x0, d_x0b, d_wk, d_wv, d_x1, d_x2, d_wm2,
              d_w1(0, 0), d_w1(0, 1), d_w1(1, 0), d_w1(1, 1), d_wo, d_w2):
        d.start()

    lane = lax.broadcasted_iota(i32, (8, 128), 1)

    def compute_mod(lo, hi):
        cf = c_s[...].astype(f32)
        sc = (cf * jax.nn.sigmoid(cf)).astype(bf16)
        sc_s[...] = jnp.broadcast_to(sc, (16, D))
        sc16 = jnp.broadcast_to(sc, (16, D))
        mod = jnp.dot(sc16, wm_s[:, lo:hi], preferred_element_type=f32)
        row = mod[0:1, :]
        for n in range((hi - lo) // 128):
            blk = jnp.broadcast_to(row[:, n * 128:(n + 1) * 128], (128, 128))
            modc_s[lo + n * 128: lo + (n + 1) * 128, :] = blk.T

    def mod_half(hf):
        lo = pl.multiple_of((1 + hf) * NM1, NM1)
        sc16 = jnp.broadcast_to(sc_s[0:1, :], (16, D))
        mod = jnp.dot(sc16, wm_s[:, pl.ds(lo, NM1)], preferred_element_type=f32)
        row = mod[0:1, :]
        plus = jnp.where(hf == 1, 1.0, 0.0)
        ridx = lax.broadcasted_iota(i32, (128, 128), 0)
        for n in range(NM1 // 128):
            blk = jnp.broadcast_to(row[:, n * 128:(n + 1) * 128], (128, 128)).T
            if n * 128 < D:
                blk = blk + jnp.where(ridx + n * 128 < D, plus, 0.0)
            modc_s[pl.ds(pl.multiple_of(lo + n * 128, 128), 128), :] = blk

    def modv(k):
        return modc_s[k * D:(k + 1) * D, :]

    def ln1(blk):
        G = D // 16
        for cc in range(TB // 128):
            col = slice(blk * TB + cc * 128, blk * TB + (cc + 1) * 128)
            acc = None
            for g in range(G):
                xf = _f32(x_s[8 * g:8 * g + 8, col])
                acc = xf if acc is None else acc + xf
            m = jnp.sum(acc, axis=0, keepdims=True) * (1.0 / D)
            acc = None
            for g in range(G):
                xc = _f32(x_s[8 * g:8 * g + 8, col]) - m
                acc = xc * xc if acc is None else acc + xc * xc
            v = jnp.sum(acc, axis=0, keepdims=True) * (1.0 / D)
            rstd = lax.rsqrt(v + EPS)
            for g in range(G):
                xc = _f32(x_s[8 * g:8 * g + 8, col]) - m
                y = xc * rstd * modc_s[D + 16 * g:D + 16 * g + 16, :] + modc_s[16 * g:16 * g + 16, :]
                hT_s[8 * g:8 * g + 8, col] = _words(y)

    def qproj(base, slot):
        wt = pltpu.bitcast(wqT_s[...], bf16)
        hv = pltpu.bitcast(hT_s[:, _ds(base, TB, TB)], bf16)
        r = jnp.dot(wt, hv, preferred_element_type=f32).astype(bf16)
        qb[slot][:, 128:128 + TB] = pltpu.bitcast(r, u32)
        qb[(slot + 1) % 3][288:864, 0:128] = qb[slot][288:864, TB:TB + 128]

    def attn_chunk(base, slot, cc, masked):
        qr = qb[slot]
        cur = pl.ds(128 + cc * 128, 128)
        prev = pl.ds(cc * 128, 128)
        for hg in range(4):
            acc = [None] * W
            for j in range(NJ):
                r = j * 32 + hg * 8
                qw = qr[r:r + 8, cur]
                q0, q1 = _unp(qw, 0), _unp(qw, 1)
                kc = qr[288 + r:288 + r + 8, cur]
                kp = qr[288 + r:288 + r + 8, prev]
                for w in range(W):
                    ks = kc if w == 0 else pltpu.roll(jnp.where(lane < 128 - DIL * w, kc, kp), DIL * w, axis=1)
                    p = q0 * _unp(ks, 0) + q1 * _unp(ks, 1)
                    acc[w] = p if acc[w] is None else acc[w] + p
            lg = acc
            if masked and cc == 0:
                pos = lane + (base + cc * 128)
                lg = [lg[0]] + [jnp.where(pos >= DIL * w, lg[w], NEG / SCALE) for w in range(1, W)]
            m = lg[0]
            for w in range(1, W):
                m = jnp.maximum(m, lg[w])
            e = [jnp.exp2((l - m) * (SCALE * LOG2E)) for l in lg]
            s = e[0]
            for w in range(1, W):
                s = s + e[w]
            rinv = 1.0 / s
            p = [x * rinv for x in e]
            for j in range(NJ):
                r = j * 32 + hg * 8
                vc = qr[576 + r:576 + r + 8, cur]
                vp = qr[576 + r:576 + r + 8, prev]
                o0 = o1 = None
                for w in range(W):
                    vs = vc if w == 0 else pltpu.roll(jnp.where(lane < 128 - DIL * w, vc, vp), DIL * w, axis=1)
                    t0 = p[w] * _unp(vs, 0)
                    t1 = p[w] * _unp(vs, 1)
                    o0 = t0 if o0 is None else o0 + t0
                    o1 = t1 if o1 is None else o1 + t1
                o_s[r:r + 8, _ds(base + cc * 128, 128)] = _words(jnp.concatenate([o0, o1], axis=0))

    def attn(base, slot, masked=False):
        for cc in range(TB // 128):
            attn_chunk(base, slot, cc, masked)

    def oproj2(base):
        wt = pltpu.bitcast(woT_s[...], bf16)
        ov = pltpu.bitcast(o_s[:, _ds(base, 2 * TB)], bf16)
        att = jnp.dot(wt, ov, preferred_element_type=f32)
        ga = modv(2)
        for cc in range(2 * TB // 128):
            c1 = _ds(base + cc * 128, 128)
            x1_s[:, c1] = pltpu.bitcast(x_s[:, c1], bf16).astype(f32) + ga * att[:, cc * 128:(cc + 1) * 128]

    def bc(v):
        return pltpu.bitcast(v, bf16)

    def ln2(blk):
        base = blk * TF
        hh = [_ln(x1_s[:, _ds(base + cc * 128, 128)], modv(4), modv(3)) for cc in range(2)]
        x11, x12, x21, x22 = hh[0][0:256], hh[0][256:512], hh[1][0:256], hh[1][256:512]
        ops = (x11 + x22, x21 + x22, x11, x22, x11 + x12, x21 - x11, x12 - x22)
        for k in range(7):
            xo_s[_ds(blk * 448 + k * 64, 64, 64), :] = pltpu.bitcast(ops[k].astype(bf16).T, u32)
        for cc in range(2):
            xr_s[_ds(blk * 128 + cc * 64, 64, 64), 0:64] = pltpu.bitcast(hh[cc][512:D].astype(bf16).T, u32)

    def ffn(blk, slot):
        base = blk * TF
        TN = 128
        xs = [bc(xo_s[_ds(blk * 448 + k * 64, 64, 64), :]) for k in range(7)]
        xr = bc(xr_s[_ds(blk * 128, 128, 128), :])[:, 0:64]
        for j in range(HF // TN):
            c1 = slice(j * TN, (j + 1) * TN)
            c2 = slice(HF + j * TN, HF + (j + 1) * TN)
            wk = (w1c_s[0:128, c1], w1_s[0:128, c1], w1c_s[128:256, c1], w1c_s[256:384, c1],
                  w1_s[128:256, c2], w1c_s[384:512, c1], w1c_s[512:640, c1])
            r1 = jnp.dot(xr, bc(w1_s[256:288, c1]), preferred_element_type=f32)
            r2 = jnp.dot(xr, bc(w1_s[256:288, c2]), preferred_element_type=f32)
            m = [jnp.dot(xs[k], bc(wk[k]), preferred_element_type=f32) for k in range(7)]
            h11 = m[0] + m[3] - m[4] + m[6] + r1[0:128]
            h12 = m[2] + m[4] + r2[0:128]
            h21 = m[1] + m[3] + r1[128:256]
            h22 = m[0] - m[1] + m[2] + m[5] + r2[128:256]
            b11 = jnp.maximum(h11, 0.0)
            b12 = jnp.maximum(h21, 0.0)
            b21 = jnp.maximum(h12, 0.0)
            b22 = jnp.maximum(h22, 0.0)
            bs = (b11 + b22, b11, b12 - b22, b21 - b11, b22, b11 + b12, b21 + b22)
            for k in range(7):
                hb_s[k * 64:(k + 1) * 64, c1] = pltpu.bitcast(bs[k].astype(bf16), u32)
        ak = (w2c_s[0:144, :], w2c_s[144:288, :], w2T_s[0:144, 0:HF], w2T_s[144:288, HF:DFF],
              w2c_s[288:432, :], w2c_s[432:576, :], w2c_s[576:720, :])
        m = [lax.dot_general(bc(ak[k]), bc(hb_s[k * 64:(k + 1) * 64, :]), (((1,), (1,)), ((), ())),
                             preferred_element_type=f32) for k in range(7)]
        cq = ((m[0] + m[3] - m[4] + m[6], m[2] + m[4]), (m[1] + m[3], m[0] - m[1] + m[2] + m[5]))
        for r in range(2):
            rr = slice(r * 288, (r + 1) * 288)
            gb = modc_s[5 * D + r * 288:5 * D + (r + 1) * 288, :]
            for cc in range(2):
                c1 = _ds(base + cc * 128, 128)
                out_s[slot, rr, cc * 128:(cc + 1) * 128] = (x1_s[rr, c1] + gb * cq[r][cc]).astype(bf16)

    def combos(dst, src, rows, signs2, c0=0, ncol=HF // 128):
        for cidx in range(ncol):
            c1 = _ds(c0 + cidx * 128, 128)
            c2 = _ds(HF + c0 + cidx * 128, 128)
            for r0 in range(0, rows, RSTEP):
                ra = slice(r0, r0 + RSTEP)
                rb = slice(rows + r0, rows + r0 + RSTEP)
                quad = [src[ra, c1], src[ra, c2], src[rb, c1], src[rb, c2]]
                val = [_f32(q) for q in quad]
                for n, (ia, ib, sgn) in enumerate(signs2):
                    rd = slice(n * rows + r0, n * rows + r0 + RSTEP)
                    dst[rd, c1] = _words(val[ia] + val[ib] if sgn > 0 else val[ia] - val[ib])

    def prep_w1(hf):
        combos(w1c_s, w1_s, 128, ((0, 3, 1), (1, 3, -1), (2, 0, -1), (0, 1, 1), (2, 3, 1)), hf * HQ, HQ // 128)

    def prep_w2():
        combos(w2c_s, w2T_s, 144, ((0, 3, 1), (2, 3, 1), (0, 1, 1), (2, 0, -1), (1, 3, -1)))

    def prep_wqkv(c0, c1, w0, w1):
        for cidx in range(c0, c1):
            ncol = 128 if cidx < 13 else 64
            t = wqkv_s[:, cidx * 128: cidx * 128 + ncol].T
            tw = pltpu.bitcast(t, u32)
            for kt in range(5):
                kw = 128 if kt < 4 else 64
                tmp_s[kt, cidx * 64: cidx * 64 + ncol // 2, 0:kw] = tw[:, kt * 128: kt * 128 + kw]
        for which in range(w0, w1):
            for j in range(NJ):
                for kt in range(5):
                    kw = 128 if kt < 4 else 64
                    v = tmp_s[kt, pl.ds(which * 288 + j, 32, stride=NJ), :]
                    wqT_s[which * 288 + j * 32: which * 288 + (j + 1) * 32, kt * 128: kt * 128 + kw] = v[:, 0:kw]

    def prep_wo():
        for nt in range(5):
            nw = 128 if nt < 4 else 64
            wof_s[nt, :, 0:nw] = wo_s[:, nt * 128: nt * 128 + nw].astype(f32)
        for nt in range(5):
            nw = 128 if nt < 4 else 64
            parts = [wof_s[nt, pl.ds(hg * 8 * DH + 2 * j + e, 8, stride=DH), :]
                     for j in range(NJ) for hg in range(4) for e in range(2)]
            pb = jnp.concatenate(parts, axis=0).astype(bf16)
            tt = pb[:, 0:nw].T
            woT_s[nt * 64: nt * 64 + nw // 2, :] = pltpu.bitcast(tt, u32)

    qb0[288:864, 0:128] = jnp.zeros((576, 128), u32)
    d_c.wait()
    d_wm1.wait()
    compute_mod(0, NM1)
    modc_s[D:2 * D, :] = modc_s[D:2 * D, :] + 1.0
    d_wq.wait()
    prep_wqkv(0, 5, 0, 1)
    d_x0.wait()
    ln1(0)
    d_x0b.wait()
    ln1(1)

    def qpart(r0, r1):
        wt = pltpu.bitcast(wqT_s[r0:r1, :], bf16)
        hv = pltpu.bitcast(hT_s[:, 0:2 * TB], bf16)
        r = pltpu.bitcast(jnp.dot(wt, hv, preferred_element_type=f32).astype(bf16), u32)
        qb0[r0:r1, 128:128 + TB] = r[:, 0:TB]
        qb1[r0:r1, 128:128 + TB] = r[:, TB:2 * TB]
        if r0 >= 288:
            qb1[r0:r1, 0:128] = qb0[r0:r1, TB:TB + 128]

    qpart(0, 144)
    d_wk.wait()
    qpart(144, 288)
    prep_wqkv(5, 9, 1, 2)
    d_wv.wait()
    d_x1.wait()
    qpart(288, 576)
    prep_wqkv(9, 14, 2, 3)
    ln1(2)
    ln1(3)
    d_x2.wait()
    qpart(576, 864)
    for blk in range(4, NB):
        ln1(blk)
    qb2[288:864, 0:128] = qb1[288:864, TB:TB + 128]

    def body(i, slot, masked=False):
        attn((i - 2) * TB, (slot + 1) % 3, masked)
        qproj(i * TB, slot)

    d_wm2.wait()

    @pl.loop(0, (NB - 2) // 3)
    def _(ii):
        i = 2 + 3 * ii
        mod_half(ii)
        body(i, 2, True)
        d_w1(ii, 0).wait()
        d_w1(ii, 1).wait()
        prep_w1(ii)
        body(i + 1, 0)
        body(i + 2, 1)

    d_wo.wait()
    prep_wo()
    attn((NB - 2) * TB, (NB - 2) % 3)
    attn((NB - 1) * TB, (NB - 1) % 3)
    oproj2(0)
    oproj2(2 * TB)
    oproj2(4 * TB)
    d_w2.wait()
    prep_w2()
    oproj2(6 * TB)
    ln2(0)

    def out_copy(b, slot):
        return pltpu.make_async_copy(out_s.at[slot], outT_hbm.at[:, _ds(b * TF, TF)], osems.at[slot])

    @pl.loop(0, NF)
    def _(i):
        slot = i % 2

        @pl.when(i >= 2)
        def _():
            out_copy(i - 2, slot).wait()
        ffn(i, slot)
        ln2(jnp.minimum(i + 1, NF - 1))
        out_copy(i, slot).start()

    out_copy(NF - 2, NF % 2).wait()
    out_copy(NF - 1, (NF - 1) % 2).wait()


@jax.jit
def pallas_adaLN_cond__sliding_local_dilated__dense_activation_relu__prompt_kernel(
        A_x, A_wqkv, A_wo, B_x, B_w1, B_w2, c, w_mod):
    xT = A_x.reshape(S, D).T
    w2T = B_w2.T
    hbm = pl.BlockSpec(memory_space=pltpu.HBM)
    VM = pltpu.VMEM
    outT = pl.pallas_call(
        _kernel,
        in_specs=[hbm] * 7,
        out_specs=hbm,
        out_shape=jax.ShapeDtypeStruct((D, S), bf16),
        scratch_shapes=[
            VM((D // 2, S), u32),
            VM((D, 3 * D), bf16),
            VM((D, D), bf16),
            VM((D // 2, DFF), u32),
            VM((D // 2, DFF), u32),
            VM((1, D), bf16),
            VM((D, 6 * D), bf16),
            VM((5, 896, 128), u32),
            VM((3 * D // 2, D), u32),
            VM((D // 2, D), u32),
            VM((6 * D, 128), f32),
            VM((D // 2, S), u32),
            VM((3 * D // 2, 128 + TB), u32), VM((3 * D // 2, 128 + TB), u32),
            VM((3 * D // 2, 128 + TB), u32),
            VM((D // 2, S), u32),
            VM((D, S), f32),
            VM((NF * 7 * 64, 256), u32),
            VM((S // 2, 128), u32),
            VM((7 * 64, HF), u32),
            VM((5 * 128, HF), u32),
            VM((5 * 144, HF), u32),
            VM((2, D, TF), bf16),
            VM((16, D), bf16),
            VM((5, D, 128), f32),
            pltpu.SemaphoreType.DMA((13,)),
            pltpu.SemaphoreType.DMA((2,)),
            pltpu.SemaphoreType.DMA((4,)),
        ],
        compiler_params=pltpu.CompilerParams(
            vmem_limit_bytes=110 * 1024 * 1024,
            flags={"XLA_TPU_EVENLY_DISTRIBUTE_CRITICAL_NODES": True},
        ),
        name="adaln_attn_ffn_kernel",
    )(xT, A_wqkv, A_wo, B_w1, w2T, c, w_mod)
    return outT.T.reshape(1, S, D)
```
